```python
import jax
import jax.numpy as jnp

def _softmax(x, axis=-1):
    return jax.nn.softmax(x, axis=axis)
def _gelu(x):
    return jax.nn.gelu(x, approximate=True)
def _silu(x):
    return jax.nn.silu(x)
def _sigmoid(x):
    return jax.nn.sigmoid(x)
def _layernorm(x, axis=-1, eps=1e-5):
    m = jnp.mean(x, axis=axis, keepdims=True)
    v = jnp.var(x, axis=axis, keepdims=True)
    return (x - m) / jnp.sqrt(v + eps)
def _scatter_add(tgt, idx, src, axis=0):
    return tgt.at[idx].add(src)
def _segment_sum(src, seg, n):
    return jax.ops.segment_sum(src, seg, n)
class _Rng:
    def __init__(self, key):
        self._k = key
    def _next(self):
        self._k, sub = jax.random.split(self._k)
        return sub
    def normal(self, shape):
        return jax.random.normal(self._next(), shape, dtype=jnp.bfloat16)
    def randint(self, lo, hi, shape):
        return jax.random.randint(self._next(), shape, lo, hi, dtype=jnp.int32)
    def uniform(self, shape, lo=0.0, hi=1.0):
        return jax.random.uniform(self._next(), shape, jnp.bfloat16, lo, hi)
    def permutation(self, n):
        return jax.random.permutation(self._next(), n)


kernel_name = 'interleave_layers__sliding_block_cached__dense_activation_gelu__decode'

def setup_inputs():
    _rng = _Rng(jax.random.key(int.from_bytes(__import__("os").urandom(4), "little")))
    _w = (lambda a: (lambda t: t.astype(jnp.bfloat16) if jnp.issubdtype(t.dtype, jnp.floating) else t)(jnp.asarray(a)))
    def _A_setup():
        B, Sq, D = 1, 1, 640
        Hq, Hkv, Sk, Dh = 32, 32, 32768, 192
        assert Hq % Hkv == 0, (Hq, Hkv)
        return {
            "x": _w((lambda *s: _rng.normal(s) * 0.05)(B, Sq, D)),
            "k_cache": _w((lambda *s: _rng.normal(s) * 0.05)(B, Hkv, Sk, Dh)),
            "v_cache": _w((lambda *s: _rng.normal(s) * 0.05)(B, Hkv, Sk, Dh)),
            "wq": _w((lambda *s: _rng.normal(s) * 0.05)(D, Hq * Dh) * (D ** -0.5)),
            "wo": _w((lambda *s: _rng.normal(s) * 0.05)(Hq * Dh, D) * ((Hq * Dh) ** -0.5)),
        }
    _A_in = _A_setup()

    def _B_setup():
        B, S, D, F = 1, 1, 640, 1536
        return {
            "x": _w((lambda *s: _rng.normal(s) * 0.05)(B, S, D)),
            "w1": _w((lambda *s: _rng.normal(s) * 0.05)(D, F) * (D ** -0.5)),
            "b1": _w((lambda *s: _rng.normal(s) * 0.05)(F) * 0.01),
            "w2": _w((lambda *s: _rng.normal(s) * 0.05)(F, D) * (F ** -0.5)),
            "b2": _w((lambda *s: _rng.normal(s) * 0.05)(D) * 0.01),
        }
    _B_in = _B_setup()

    return {
        "A_x": _A_in["x"],
        "A_k_cache": _A_in["k_cache"],
        "A_v_cache": _A_in["v_cache"],
        "A_wq": _A_in["wq"],
        "A_wo": _A_in["wo"],
        "B_x": _B_in["x"],
        "B_w1": _B_in["w1"],
        "B_b1": _B_in["b1"],
        "B_w2": _B_in["w2"],
        "B_b2": _B_in["b2"],
    }

def reference(A_x, A_k_cache, A_v_cache, A_wq, A_wo, B_x, B_w1, B_b1, B_w2, B_b2):
    def _A_ref(x, k_cache, v_cache, wq, wo):
        B, Sq, D = x.shape
        Hq, Dh = 32, 192
        Hkv, Sk = k_cache.shape[1], k_cache.shape[2]
        W = min(4096, max(256, Sk // 4))
        rep = Hq // Hkv
        q = (lambda x, *d: x.transpose(*d))((x @ wq).reshape(B, Sq, Hq, Dh), 0, 2, 1, 3)
        k = jnp.repeat(k_cache[:, :, Sk - W:, :], rep, axis=1)
        v = jnp.repeat(v_cache[:, :, Sk - W:, :], rep, axis=1)
        scores = jnp.einsum("bhqd,bhkd->bhqk", q, k) * (Dh ** -0.5)
        p = _softmax(scores, axis=-1)
        o = jnp.einsum("bhqk,bhkd->bhqd", p, v)
        return (lambda x, *d: x.transpose(*d))(o, 0, 2, 1, 3).reshape(B, Sq, Hq * Dh) @ wo

    def _B_ref(x, w1, b1, w2, b2):
        h = jnp.einsum("bsd,df->bsf", x, w1) + b1
        h = _gelu(h)
        return jnp.einsum("bsf,fd->bsd", h, w2) + b2

    x = A_x
    x = x + _A_ref(_layernorm(x, axis=-1), A_k_cache, A_v_cache, A_wq, A_wo)
    x = x + _B_ref(_layernorm(x, axis=-1), B_w1, B_b1, B_w2, B_b2)
    x = x + _A_ref(_layernorm(x, axis=-1), A_k_cache, A_v_cache, A_wq, A_wo)
    x = x + _B_ref(_layernorm(x, axis=-1), B_w1, B_b1, B_w2, B_b2)
    return x
```

```python
import jax
import jax.numpy as jnp
from jax import lax
import jax.experimental.pallas as pl
import jax.experimental.pallas.tpu as pltpu

_HQ, _DH = 32, 192
_LANES = 128
_GH = 16
_GR = _GH * _DH
_BF, _F32 = jnp.bfloat16, jnp.float32


def _layernorm(x):
    m = jnp.mean(x, axis=-1, keepdims=True)
    d = x - m
    v = jnp.mean(d * d, axis=-1, keepdims=True)
    return d / jnp.sqrt(v + 1e-5)


def _gelu(x):
    c = 0.7978845608028654
    return 0.5 * x * (1.0 + jnp.tanh(c * (x + 0.044715 * (x * x * x))))


def _kernel(x_ref, b1_ref, b2_ref, k_hbm, v_hbm, wq_hbm, wo_hbm, w1_hbm, w2_hbm, o_ref,
            kbuf, vbuf, wq, wo, w1, w2, s_ref, p_ref, ksem, vsem, wsem, *, start, nt):
    inflight = 4

    def kv_copy(i):
        def mk(src, dst, sem, c):
            off = pl.multiple_of(start + c * _LANES, _LANES)
            return pltpu.make_async_copy(src.at[:, pl.ds(off, _LANES)], dst.at[c], sem.at[c])
        return mk

    def kcp(c):
        off = pl.multiple_of(start + c * _LANES, _LANES)
        return pltpu.make_async_copy(k_hbm.at[:, pl.ds(off, _LANES)], kbuf.at[c], ksem.at[c])

    def vcp(c):
        off = pl.multiple_of(start + c * _LANES, _LANES)
        return pltpu.make_async_copy(v_hbm.at[:, pl.ds(off, _LANES)], vbuf.at[c], vsem.at[c])

    wcp = [pltpu.make_async_copy(s, d, wsem.at[i]) for i, (s, d) in enumerate(
        ((wq_hbm, wq), (wo_hbm, wo), (w1_hbm, w1), (w2_hbm, w2)))]

    wcp[0].start()
    for c in range(inflight):
        kcp(c).start()

    row = lax.broadcasted_iota(jnp.int32, (_GH, _GR), 0)
    col = lax.broadcasted_iota(jnp.int32, (_GH, _GR), 1)
    diag = (col >= row * _DH) & (col < (row + 1) * _DH)
    ng = _HQ // _GH

    def rb(a):
        return a.astype(_BF).astype(_F32)

    x = jnp.broadcast_to(x_ref[...].astype(_F32), (16, x_ref.shape[-1]))
    for layer in range(2):
        first = layer == 0
        if first:
            wcp[0].wait()
        q = jnp.dot(_layernorm(x).astype(_BF), wq[...], preferred_element_type=_F32)
        qbd = [jnp.where(diag, q[:, g * _GR:(g + 1) * _GR], 0.0).astype(_BF) for g in range(ng)]

        def k_body(c, m):
            if first:
                kcp(c).wait()

                @pl.when(c + inflight < nt)
                def _():
                    kcp(c + inflight).start()

                @pl.when(c + inflight >= nt)
                def _():
                    vcp(c + inflight - nt).start()
            s = jnp.concatenate(
                [jnp.dot(qbd[g], kbuf[c, g * _GR:(g + 1) * _GR, :], preferred_element_type=_F32)
                 for g in range(ng)], axis=0) * (_DH ** -0.5)
            s_ref[c] = s
            return jnp.maximum(m, s)

        m = lax.fori_loop(0, nt, k_body, jnp.full((_HQ, _LANES), -jnp.inf, _F32))
        m = jnp.max(m, axis=-1, keepdims=True)
        e = jnp.exp(s_ref[...] - m[None])
        l = jnp.sum(jnp.sum(e, axis=0), axis=-1, keepdims=True)
        p_ref[...] = (e / l[None]).astype(_BF)

        def v_body(c, acc):
            if first:
                vcp(c).wait()

                @pl.when(c + inflight < nt)
                def _():
                    vcp(c + inflight).start()

                for i in range(3):
                    @pl.when(c + inflight - nt == i)
                    def _():
                        wcp[1 + i].start()
            return tuple(
                acc[g] + lax.dot_general(p_ref[c, g * _GH:(g + 1) * _GH, :], vbuf[c, g * _GR:(g + 1) * _GR, :],
                                         (((1,), (1,)), ((), ())), preferred_element_type=_F32)
                for g in range(ng))

        acc = lax.fori_loop(0, nt, v_body, tuple(jnp.zeros((_GH, _GR), _F32) for _ in range(ng)))
        o = jnp.concatenate([jnp.where(diag, a, 0.0).astype(_BF) for a in acc], axis=1)
        if first:
            wcp[1].wait()
        a = jnp.sum(jnp.dot(o, wo[...], preferred_element_type=_F32), axis=0, keepdims=True)
        x = rb(x + rb(a))
        if first:
            wcp[2].wait()
        h = jnp.dot(_layernorm(x).astype(_BF), w1[...], preferred_element_type=_F32)
        h = _gelu(rb(rb(h) + b1_ref[...].astype(_F32)))
        if first:
            wcp[3].wait()
        f = jnp.dot(h.astype(_BF), w2[...], preferred_element_type=_F32)
        x = rb(x + rb(rb(f) + b2_ref[...].astype(_F32)))
    o_ref[...] = x[0:1].astype(o_ref.dtype)


@jax.jit
def pallas_interleave_layers__sliding_block_cached__dense_activation_gelu__decode_kernel(
    A_x: jax.Array,
    A_k_cache: jax.Array,
    A_v_cache: jax.Array,
    A_wq: jax.Array,
    A_wo: jax.Array,
    B_x: jax.Array,
    B_w1: jax.Array,
    B_b1: jax.Array,
    B_w2: jax.Array,
    B_b2: jax.Array,
):
    import functools
    d = A_x.shape[-1]
    sk = A_k_cache.shape[2]
    w = min(4096, max(256, sk // 4))
    nt = w // _LANES
    rows = _HQ * _DH
    kt = jnp.swapaxes(A_k_cache, 2, 3).reshape(rows, sk)
    vt = jnp.swapaxes(A_v_cache, 2, 3).reshape(rows, sk)
    vm = pl.BlockSpec(memory_space=pltpu.VMEM)
    hbm = pl.BlockSpec(memory_space=pl.ANY)
    out = pl.pallas_call(
        functools.partial(_kernel, start=sk - w, nt=nt),
        out_shape=jax.ShapeDtypeStruct((1, d), A_x.dtype),
        in_specs=[vm, vm, vm] + [hbm] * 6,
        out_specs=vm,
        scratch_shapes=[
            pltpu.VMEM((nt, rows, _LANES), _BF),
            pltpu.VMEM((nt, rows, _LANES), _BF),
            pltpu.VMEM(A_wq.shape, _BF),
            pltpu.VMEM(A_wo.shape, _BF),
            pltpu.VMEM(B_w1.shape, _BF),
            pltpu.VMEM(B_w2.shape, _BF),
            pltpu.VMEM((nt, _HQ, _LANES), _F32),
            pltpu.VMEM((nt, _HQ, _LANES), _BF),
            pltpu.SemaphoreType.DMA((nt,)),
            pltpu.SemaphoreType.DMA((nt,)),
            pltpu.SemaphoreType.DMA((4,)),
        ],
        compiler_params=pltpu.CompilerParams(vmem_limit_bytes=126 * 2**20),
    )(A_x.reshape(1, d), B_b1.reshape(1, -1), B_b2.reshape(1, -1), kt, vt, A_wq, A_wo, B_w1, B_w2)
    return out.reshape(A_x.shape)
```

```python
import functools

import jax
import jax.numpy as jnp
from jax import lax
import jax.experimental.pallas as pl
import jax.experimental.pallas.tpu as pltpu

_HQ, _DH = 32, 192
_L = 128
_GH = 4
_NG = _HQ // _GH
_GR = _GH * _DH
_KT = _GR // _L
_BF, _F32, _U32 = jnp.bfloat16, jnp.float32, jnp.uint32

CFG = dict(nj=2, every=5, lag=7, slag=5, nx=2, end=16, smlag=6, sms=1, lend=16, tu=4, nl=2, sm2=9, fst=16, fs=1, pf=0, fa=0, aa=1, pl=0, pad=0)


def _layernorm(x):
    m = jnp.mean(x, axis=-1, keepdims=True)
    d = x - m
    v = jnp.mean(d * d, axis=-1, keepdims=True)
    return d / jnp.sqrt(v + 1e-5)


def _gelu(x):
    c = 0.7978845608028654
    return 0.5 * x * (1.0 + jnp.tanh(c * (x + 0.044715 * (x * x * x))))


def _rb(a):
    return a.astype(_BF).astype(_F32)


def _bf(a):
    return pltpu.bitcast(a, _BF)


def _lhs(a):
    return jnp.concatenate([a, a], axis=0).astype(_BF)


def _mm(a, b):
    return jnp.dot(a, b, preferred_element_type=_F32)[:8]


def _kernel(x_ref, b1_ref, b2_ref, k_hbm, v_hbm, wq_hbm, wo_hbm, w1_hbm, w2_hbm, o_ref,
            ar_b, vb_b, wq_b, wo_b, w1_b, w2_b, ps, es, u_ref, q_ref, ol_ref, oacc, ox_ref, xa_ref, z_ref, sem, *, start, nt):
    ar, vb, wq, wo, w1, w2 = (r.bitcast(_U32) for r in (ar_b, vb_b, wq_b, wo_b, w1_b, w2_b))
    nj, every, lag, slag, nx, end, smlag = (CFG[k] for k in ("nj", "every", "lag", "slag", "nx", "end", "smlag"))
    d = x_ref.shape[-1]
    hr, hl = _GR // 16, _L // 16
    vx0 = _NG * hr
    hx = nx * hl
    dm0 = vx0 + _NG * hx

    def copies(g):
        out = []

        def cp(src, r0, c0, dst, d0, n, i):
            nc = src.shape[2] - c0
            for h in range(2):
                out.append(pltpu.make_async_copy(
                    src.at[pl.ds(r0, n), h, pl.ds(c0, nc)],
                    dst.at[pl.ds(d0, n), pl.ds(0, nc), pl.ds(8 * h, 8)], sem.at[2 * i + h]))

        if g < 0:
            cp(wq_hbm, 0, 0, wq_b, 0, d // 16, 3)
        if g + 1 < _NG:
            cp(k_hbm, (g + 1) * hr, start, ar_b, (g + 1) * hr, hr, 3 * g + 7)
        if 0 <= g < _NG:
            cp(v_hbm, g * hr, start, vb_b, g * (hr - hx), hr - hx, 3 * g + 5)
            cp(v_hbm, (g + 1) * hr - hx, start, ar_b, vx0 + g * hx, hx, 3 * g + 6)
        if g == 0:
            cp(wo_hbm, 0, 0, wo_b, 0, _NG * hr, 0)
        if g == _NG:
            cp(w1_hbm, 0, 0, w1_b, 0, w1_b.shape[0], 1)
        if g == _NG + 1:
            cp(w2_hbm, 0, 0, w2_b, 0, w2_b.shape[0], 2)
        return out

    def mat(ref, r0, n, cols):
        return jnp.concatenate([_bf(ref[pl.ds(r0, n), c].reshape(8 * n, _L)) for c in cols], axis=1)

    def advance(g):
        for c in copies(g):
            c.wait()
        for c in copies(g + 2):
            c.start()

    for g in (-1, 0):
        for c in copies(g):
            c.start()

    oacc[...] = jnp.zeros_like(oacc)
    ox_ref[...] = jnp.zeros_like(ox_ref)
    z_ref[0] = 0
    z_ref[1] = 0

    def set_q(q):
        row = lax.broadcasted_iota(jnp.int32, q.shape, 0)
        col = lax.broadcasted_iota(jnp.int32, q.shape, 1)
        diag = (col >= row * _DH) & (col < (row + 1) * _DH)
        q_ref[...] = pltpu.bitcast(_lhs(jnp.where(diag, q, 0.0)), _U32)

    def exp_sum(s_of, m):
        l = None
        for c in range(nt):
            e = jnp.exp(s_of(c) - m)
            es[c] = e
            l = e if l is None else l + e
        r = jnp.broadcast_to(1.0 / jnp.sum(l, axis=-1, keepdims=True), (8, _L))
        es[nt] = r
        return r

    def finish_o(t, slot):
        if t < _KT - nx:
            a = oacc[pl.ds(pl.multiple_of(slot * _GR + t * _L, 8), _L), :].T
        else:
            a = ox_ref[t - (_KT - nx)]
            head = (t * _L + lax.broadcasted_iota(jnp.int32, a.shape, 1)
                    - _DH * lax.broadcasted_iota(jnp.int32, a.shape, 0))
            a = jnp.where((head >= 0) & (head < _DH), a, 0.0)
        o = jnp.sum(a, axis=0, keepdims=True)
        ol_ref[:, t * _L:(t + 1) * _L] = pltpu.bitcast(_lhs(jnp.broadcast_to(o, (8, _L))), _U32)
        return jnp.broadcast_to(o, (8, _L))

    def group_body(first, g, last=False):
        @pl.loop(0, first)
        def _(_):
            for j in ([_NG - 1] if last else range(_NG - 1)):
                pl.when(g == j)(functools.partial(advance, j))

            tu = CFG["tu"]

            @pl.loop(0, nt // tu)
            def _(cb):
                at = [(vx0 + g * hx + t * hl, cb * tu + c) for c in range(tu) for t in range(nx)]
                tr = [mat(ar, r, hl, [c]).T for r, c in at]
                for (r, c), a in zip(at, tr):
                    ar[pl.ds(r, hl), c] = pltpu.bitcast(a, _U32).reshape(hl, 8, _L)

        z, z2 = z_ref[0], z_ref[1]
        prow = pl.multiple_of(8 * z, 8)
        srow = pl.multiple_of(8 + 8 * z, 8)
        krow = (g + 1) * hr
        orow = jnp.maximum(g - 1, 0) * hr
        qcol = jnp.minimum(g + 2, _NG - 1) * _KT
        for c in range(nt):
            ps[c, pl.ds(prow, 8), :] = es[c] * es[nt]

        tiles = []
        karr, xarr = ar.at[pl.ds(krow, hr)], ar.at[pl.ds(vx0 + g * hx, hx)]
        varr = vb.at[pl.ds(g * (hr - hx), hr - hx)]
        for cb in range(0, 0 if last else nt, 4):
            for t in range(_KT):
                for c in range(cb, cb + 4):
                    tiles.append((karr, t, c, lambda t=t: _bf(q_ref[:, t * _L:(t + 1) * _L]), False, ("s", c)))
        n_k = len(tiles)
        for c in range(nt):
            for t in range(nx):
                tiles.append((xarr, t, c, lambda c=c: _lhs(ps[c, pl.ds(prow, 8), :]), False, ("x", t)))
        for n in range(0 if last else _KT):
            for t in range(d // _L):
                tiles.append((wq.at[:, pl.ds(qcol, _KT)], t, n, lambda t=t: _bf(u_ref[:, t * _L:(t + 1) * _L]), False, ("q", n)))
        for n in range(d // _L):
            for t in range(_KT):
                tiles.append((wo.at[pl.ds(orow, hr)], t, n, lambda t=t: _bf(ol_ref[:, t * _L:(t + 1) * _L]),
                              False, ("o", n)))
        left = {}
        for tl in tiles:
            left[tl[5]] = left.get(tl[5], 0) + 1
        pend, res, qs = [], {}, {}

        def retire(n):
            while len(pend) > n:
                batch = pend.pop(0)
                for key, r in batch:
                    res[key] = r if key not in res else res[key] + r
                    left[key] -= 1
                    if left[key]:
                        continue
                    kind, i = key
                    cols = slice(i * _L, (i + 1) * _L)
                    if kind == "s":
                        sc = res[key] * (_DH ** -0.5)
                        ps[i, pl.ds(srow, 8), :] = sc
                        res["m"] = sc if i == 0 else jnp.maximum(res["m"], sc)
                    elif kind == "q":
                        qs[i] = res[key]
                        if len(qs) == _KT:
                            set_q(jnp.concatenate([qs[j] for j in range(_KT)], axis=1))
                    elif kind == "o":
                        xa_ref[:, cols] += jnp.where(g > 0, res[key], 0.0)
                    else:
                        ox_ref[i] = res[key]
                key = batch[-1][0]
                if CFG["aa"] or left[key]:
                    ps[nt + z2, 8:16, :] = res[key]

        tasks = []
        for b in range(0, len(tiles), 4):
            bt = tiles[b:b + 4]
            rows = [[None] * 8 for _ in bt]

            def task(j, bt=bt, rows=rows):
                for jj in (j, j - 1):
                    for r, (ref, t, c, *_) in zip(rows, bt):
                        r[jj] = ref[t * hl + jj, c]
                if j == 1:
                    out = []
                    for r, (_, _, _, lhs, xp, key) in zip(rows, bt):
                        w = _bf(jnp.concatenate(r, axis=0))
                        out.append((key, lax.dot_general(lhs(), w, (((1,), (1 if xp else 0,)), ((), ())),
                                                         preferred_element_type=_F32)[:8]))
                    pend.append(out)

            for j in (7, 5, 3, 1):
                tasks.append((2 if bt[-1][4] else 1, functools.partial(task, j), {tl[5][0] for tl in bt}))

        def anchor(v):
            ps[nt + z2, 0:8, :] = v

        def sm_max():
            assert left["s", nt - 1] == 0
            res["mx"] = jnp.broadcast_to(jnp.max(res["m"], axis=-1, keepdims=True), (8, _L))

        def sm_exp(c):
            if c >= 4 and c % 2 == 0:
                anchor(res["l", c - 4])
            e = jnp.exp(ps[c, pl.ds(srow, 8), :] - res["mx"])
            es[c] = e
            res["l", c] = e if c == 0 else res["l", c - 1] + e
            if c == nt - 1:
                es[nt] = jnp.broadcast_to(1.0 / jnp.sum(res["l", c], axis=-1, keepdims=True), (8, _L))

        def fin(t):
            if t and CFG["fa"]:
                anchor(res["f"])
            if t < _KT:
                res["f"] = finish_o(t, 1 - g % 2)

        extra = {}
        if not last:
            extra[n_k + 4 * smlag] = sm_max
            for c in range(nt):
                extra[n_k + 4 * CFG["sm2"] + CFG["sms"] * c] = functools.partial(sm_exp, c)
        for t in range(_KT + 1):
            extra[4 + (1 if last else CFG["fst"]) * t] = functools.partial(fin, t)
        for i in sorted(extra, reverse=True):
            tasks.insert(i, (0, extra[i], ()))

        blocks = [(r, c) for r in range(0, hr - hx, nj) for c in range(nt)]
        total, span = sum(w for w, _, _ in tasks), len(blocks) - (CFG["lend"] if last else end)
        hist, done, acc, late = [], 0, None, []
        for step, (r, c) in enumerate(blocks):
            if step % every == 0:
                run = []
                while tasks and done * span < (step + every) * total:
                    run.append(tasks.pop(0))
                    done += run[-1][0]
                if len(hist) > lag:
                    old = pltpu.bitcast(hist[-1 - lag], _U32)
                    kinds = set().union(*(k for _, _, k in run))
                    for a in range(0, 2 * nj, CFG["fs"]):
                        v = old[8 * a:8 * a + 8]
                        if kinds & {"s", "x"}:
                            ar[dm0 + z, a] = v
                        if "q" in kinds:
                            wq[d // 16 + z, a] = v
                        if "o" in kinds:
                            wo[_NG * hr + z + a // 4, a % 4] = v
                    if CFG["pf"]:
                        ps[nt + 1 + z2, 0:8, :] = hist[-1 - lag + CFG["pl"]][:8]
                retire(slag)
                for _, fn, _ in run:
                    fn()
            pb = ps[c, pl.ds(prow + (16 * r) // _DH, 8, stride=0), :]
            pb = jnp.concatenate([pb] * (2 * nj), axis=0)
            vv = mat(varr, r, nj, [c])
            t = vv.astype(_F32) * pb
            acc = t if acc is None else acc + t
            hist.append(acc)
            if c == nt - 1:
                late.append((r, acc))
                acc = None
                r0, a0 = late.pop()
                oacc[pl.ds(pl.multiple_of(_GR * (g % 2) + 16 * r0, 8), 16 * nj), :] = a0
        assert not tasks
        retire(0)

    def layer(i, x):
        first = jnp.maximum(1 - i, 0)
        u = _lhs(_layernorm(x))
        u_ref[...] = pltpu.bitcast(u, _U32)
        xa_ref[...] = jnp.zeros_like(xa_ref)
        pl.loop(0, first)(lambda _: advance(-1))
        set_q(_mm(u, mat(wq, 0, d // 16, range(_KT))))
        q1 = _mm(u, mat(wq, 0, d // 16, range(_KT, 2 * _KT)))
        s = _mm(_bf(q_ref[...]), mat(ar, 0, hr, range(nt))) * (_DH ** -0.5)
        exp_sum(lambda c: s[:, c * _L:(c + 1) * _L], jnp.max(s, axis=-1, keepdims=True))
        set_q(q1)

        lax.fori_loop(0, _NG - 1, lambda g, _: group_body(first, g), None)
        group_body(first, _NG - 1 + z_ref[0], last=True)

        for t in range(_KT):
            finish_o(t, (_NG - 1) % 2)
        a = xa_ref[...] + _mm(_bf(ol_ref[...]), mat(wo, (_NG - 1) * hr, hr, range(d // _L)))
        x = _rb(x + _rb(a))
        pl.when(first > 0)(lambda: advance(_NG))
        h = _mm(_lhs(_layernorm(x)), mat(w1, 0, w1.shape[0], range(w1.shape[1])))
        h = _gelu(_rb(_rb(h) + b1_ref[...].astype(_F32)[None]))
        pl.when(first > 0)(lambda: advance(_NG + 1))
        f = _mm(_lhs(h), mat(w2, 0, w2.shape[0], range(w2.shape[1])))
        return _rb(x + _rb(_rb(f) + b2_ref[...].astype(_F32)[None]))

    x = lax.fori_loop(0, CFG["nl"], layer, jnp.broadcast_to(x_ref[0].astype(_F32), (8, d)))
    o_ref[0] = x[0:1].astype(o_ref.dtype)


@jax.jit
def pallas_interleave_layers__sliding_block_cached__dense_activation_gelu__decode_kernel(
    A_x: jax.Array,
    A_k_cache: jax.Array,
    A_v_cache: jax.Array,
    A_wq: jax.Array,
    A_wo: jax.Array,
    B_x: jax.Array,
    B_w1: jax.Array,
    B_b1: jax.Array,
    B_w2: jax.Array,
    B_b2: jax.Array,
):
    d, f = B_w1.shape
    sk = A_k_cache.shape[2]
    w = min(4096, max(256, sk // 4))
    rows = _HQ * _DH
    kt = jnp.swapaxes(A_k_cache, 2, 3).reshape(rows, sk)
    vt = jnp.swapaxes(A_v_cache, 2, 3).reshape(rows, sk)

    def tiled(a):
        r, c = a.shape
        return a.reshape(r // 16, 2, 8, c // _L, _L).transpose(0, 1, 3, 2, 4)

    def buf(r, c, extra=0, pad=0):
        return pltpu.VMEM((r // 16 + extra, c // _L + pad, 16, _L), _BF)

    vm = pl.BlockSpec(memory_space=pltpu.VMEM)
    hbm = pl.BlockSpec(memory_space=pl.ANY)
    return pl.pallas_call(
        functools.partial(_kernel, start=(sk - w) // _L, nt=w // _L),
        out_shape=jax.ShapeDtypeStruct(A_x.shape, A_x.dtype),
        in_specs=[vm, vm, vm] + [hbm] * 6,
        out_specs=vm,
        scratch_shapes=[
            buf(rows + CFG["nx"] * _NG * _L, w, 1, CFG["pad"]),
            buf(rows - CFG["nx"] * _NG * _L, w, 0, CFG["pad"]),
            buf(d, rows, 1),
            buf(rows, d, 2),
            buf(d, f),
            buf(f, d),
            pltpu.VMEM((w // _L + 2, 16, _L), _F32),
            pltpu.VMEM((w // _L + 1, 8, _L), _F32),
            pltpu.VMEM((8, d), _U32),
            pltpu.VMEM((8, _GR), _U32),
            pltpu.VMEM((8, _GR), _U32),
            pltpu.VMEM((2 * _GR, _L), _F32),
            pltpu.VMEM((CFG["nx"], 8, _L), _F32),
            pltpu.VMEM((8, d), _F32),
            pltpu.SMEM((2,), jnp.int32),
            pltpu.SemaphoreType.DMA((6 * _NG + 8,)),
        ],
        compiler_params=pltpu.CompilerParams(vmem_limit_bytes=126 * 2**20),
        name="attn_ffn_x2",
    )(A_x, B_b1, B_b2, *map(tiled, (kt, vt, A_wq, A_wo, B_w1, B_w2)))
```

```python
import functools

import jax
import jax.numpy as jnp
from jax import lax
import jax.experimental.pallas as pl
import jax.experimental.pallas.tpu as pltpu

_HQ, _DH = 32, 192
_L = 128
_GH = 4
_NG = _HQ // _GH
_GR = _GH * _DH
_KT = _GR // _L
_BF, _F32, _U32 = jnp.bfloat16, jnp.float32, jnp.uint32

_NX = 2
_XC, _XL = 32, 64
_NJ = 2
_EVERY, _EVERY_L = 6, 8
_END, _END_L = 16, 4
_LAG, _RETIRE = 8, 5
_SM_MAX, _SM_EXP = 6, 8


def _layernorm(x):
    m = jnp.mean(x, axis=-1, keepdims=True)
    d = x - m
    v = jnp.mean(d * d, axis=-1, keepdims=True)
    return d, jnp.broadcast_to(1.0 / jnp.sqrt(v + 1e-5), (x.shape[0], _L))


def _gelu(x):
    c = 0.7978845608028654
    return 0.5 * x * (1.0 + jnp.tanh(c * (x + 0.044715 * (x * x * x))))


def _rb(a):
    return a.astype(_BF).astype(_F32)


def _bf(a):
    return pltpu.bitcast(a, _BF)


def _lhs(a):
    return jnp.concatenate([a, a], axis=0).astype(_BF)


def _mm(a, b):
    return jnp.dot(a, b, preferred_element_type=_F32)[:8]


def _kernel(x_ref, b1_ref, b2_ref, k_hbm, v_hbm, wq_hbm, wo_hbm, w1_hbm, w2_hbm, o_ref,
            ar_b, vb_b, wq_b, wo_b, w1_b, w2_b, ps, es, u_ref, q_ref, ol_ref, oacc, ox_ref, xa_ref, z_ref, sem, *, start, nt):
    ar, vb, wq, wo, w1, w2 = (r.bitcast(_U32) for r in (ar_b, vb_b, wq_b, wo_b, w1_b, w2_b))
    nj, nx, lag = _NJ, _NX, _LAG
    d = x_ref.shape[-1]
    hr, hl = _GR // 16, _L // 16
    vx0 = _NG * hr
    hx = nx * hl
    dm0 = vx0 + _NG * hx

    w2a = w2_b.shape[0] - 2 * hl

    def copies(g):
        out = []

        def cp(src, r0, c0, dst, d0, n, i):
            nc = src.shape[2] - c0
            for h in range(2):
                out.append(pltpu.make_async_copy(
                    src.at[pl.ds(r0, n), h, pl.ds(c0, nc)],
                    dst.at[pl.ds(d0, n), pl.ds(0, nc), pl.ds(8 * h, 8)], sem.at[2 * i + h]))

        if g < 0:
            cp(wq_hbm, 0, 0, wq_b, 0, d // 16, 3)
        if g + 1 < _NG:
            cp(k_hbm, (g + 1) * hr, start, ar_b, (g + 1) * hr, hr, 3 * g + 7)
        if 0 <= g < _NG:
            cp(v_hbm, g * hr, start, vb_b, g * (hr - hx), hr - hx, 3 * g + 5)
            cp(v_hbm, (g + 1) * hr - hx, start, ar_b, vx0 + g * hx, hx, 3 * g + 6)
        if g == 0:
            cp(wo_hbm, 0, 0, wo_b, 0, _NG * hr, 0)
        if g == _NG:
            cp(w1_hbm, 0, 0, w1_b, 0, w1_b.shape[0], 1)
        if g == _NG + 1:
            cp(w2_hbm, 0, 0, w2_b, 0, w2a, 2)
        if g == _NG + 2:
            cp(w2_hbm, w2a, 0, w2_b, w2a, w2_b.shape[0] - w2a, 3 * _NG + 4)
        return out

    def mat(ref, r0, n, cols):
        return jnp.concatenate([_bf(ref[pl.ds(r0, n), c].reshape(8 * n, _L)) for c in cols], axis=1)

    def advance(g):
        for c in copies(g):
            c.wait()
        for c in copies(g + 2):
            c.start()

    for g in (-1, 0):
        for c in copies(g):
            c.start()

    oacc[...] = jnp.zeros_like(oacc)
    ox_ref[...] = jnp.zeros_like(ox_ref)
    z_ref[0] = 0
    z_ref[1] = 0

    def set_q(q):
        q = q * jnp.concatenate([es[nt + 1]] * _KT, axis=1)
        row = lax.broadcasted_iota(jnp.int32, q.shape, 0)
        col = lax.broadcasted_iota(jnp.int32, q.shape, 1)
        diag = (col >= row * _DH) & (col < (row + 1) * _DH)
        q_ref[...] = pltpu.bitcast(_lhs(jnp.where(diag, q, 0.0)), _U32)

    def exp_sum(s_of, m):
        l = None
        for c in range(nt):
            e = jnp.exp(s_of(c) - m)
            es[c] = e
            l = e if l is None else l + e
        r = jnp.broadcast_to(1.0 / jnp.sum(l, axis=-1, keepdims=True), (8, _L))
        es[nt] = r
        return r

    def on_mxu(t, last):
        return min(max((_XL if last else _XC) - (_KT - 1 - t) * nt, 0), nt)

    def finish_o(t, slot, last):
        a = None
        if on_mxu(t, last) < nt:
            a = oacc[pl.ds(pl.multiple_of(slot * _GR + t * _L, 8), _L), :].T
            a = jnp.sum(a.reshape(_L // 8, 8, _L), axis=0)
        if on_mxu(t, last):
            head = (t * _L + lax.broadcasted_iota(jnp.int32, (8, _L), 1)
                    - _DH * lax.broadcasted_iota(jnp.int32, (8, _L), 0))
            b = jnp.where((head >= 0) & (head < _DH), ox_ref[t - (_KT - nx)], 0.0)
            a = b if a is None else a + b
        o = jnp.sum(a, axis=0, keepdims=True)
        ol_ref[:, t * _L:(t + 1) * _L] = pltpu.bitcast(_lhs(jnp.broadcast_to(o, (8, _L))), _U32)

    def group_body(first, g, last=False):
        @pl.loop(0, first)
        def _(_):
            for j in ([_NG - 1] if last else range(_NG - 1)):
                pl.when(g == j)(functools.partial(advance, j))

            tu = 8

            @pl.loop(0, (_XL if last else _XC) // tu)
            def _(cb):
                at = [(vx0 + g * hx + (nx - 1 - (cb * tu) // nt) * hl, (cb * tu) % nt + c) for c in range(tu)]
                tr = [mat(ar, r, hl, [c]).T for r, c in at]
                for (r, c), a in zip(at, tr):
                    ar[pl.ds(r, hl), c] = pltpu.bitcast(a, _U32).reshape(hl, 8, _L)

        z, z2 = z_ref[0], z_ref[1]
        prow = pl.multiple_of(8 * z, 8)
        srow = pl.multiple_of(8 + 8 * z, 8)
        krow = (g + 1) * hr
        orow = jnp.maximum(g - 1, 0) * hr
        qcol = jnp.minimum(g + 2, _NG - 1) * _KT
        for c in range(nt):
            ps[c, pl.ds(prow, 8), :] = es[c] * es[nt]

        tiles = []
        karr, xarr = ar.at[pl.ds(krow, hr)], ar.at[pl.ds(vx0 + g * hx, hx)]
        varr = vb.at[pl.ds(g * (hr - hx), hr - hx)]
        for cb in range(0, 0 if last else nt, 4):
            for t in range(_KT):
                for c in range(cb, cb + 4):
                    tiles.append((karr, t, c, lambda t=t: _bf(q_ref[:, t * _L:(t + 1) * _L]), ("s", c)))
        n_k = len(tiles)
        for c in range(nt):
            for t in range(nx):
                if c < on_mxu(_KT - nx + t, last):
                    tiles.append((xarr, t, c, lambda c=c: _lhs(ps[c, pl.ds(prow, 8), :]), ("x", t)))
        for n in range(0 if last else _KT):
            for t in range(d // _L):
                tiles.append((wq.at[:, pl.ds(qcol, _KT)], t, n, lambda t=t: _bf(u_ref[:, t * _L:(t + 1) * _L]), ("q", n)))
        for n in range(d // _L):
            for t in range(_KT):
                tiles.append((wo.at[pl.ds(orow, hr)], t, n, lambda t=t: _bf(ol_ref[:, t * _L:(t + 1) * _L]),
                              ("o", n)))
        left = {}
        for tl in tiles:
            left[tl[4]] = left.get(tl[4], 0) + 1
        pend, res, qs = [], {}, {}

        def retire(n):
            while len(pend) > n:
                batch = pend.pop(0)
                for key, r in batch:
                    res[key] = r if key not in res else res[key] + r
                    left[key] -= 1
                    if left[key]:
                        continue
                    kind, i = key
                    cols = slice(i * _L, (i + 1) * _L)
                    if kind == "s":
                        sc = res[key] * (_DH ** -0.5)
                        ps[i, pl.ds(srow, 8), :] = sc
                        res["m"] = sc if i == 0 else jnp.maximum(res["m"], sc)
                    elif kind == "q":
                        qs[i] = res[key]
                        if len(qs) == _KT:
                            set_q(jnp.concatenate([qs[j] for j in range(_KT)], axis=1))
                    elif kind == "o":
                        xa_ref[:, cols] += jnp.where(g > 0, res[key], 0.0)
                    else:
                        ox_ref[i] = res[key]
                key = batch[-1][0]
                ps[nt + z2, 8:16, :] = res[key]

        tasks = []
        for b in range(0, len(tiles), 4):
            bt = tiles[b:b + 4]
            rows = [[None] * 8 for _ in bt]

            def task(j, bt=bt, rows=rows):
                for jj in (j, j - 1):
                    for r, (ref, t, c, *_) in zip(rows, bt):
                        r[jj] = ref[t * hl + jj, c]
                if j == 1:
                    out = []
                    for r, (_, _, _, lhs, key) in zip(rows, bt):
                        w = _bf(jnp.concatenate(r, axis=0))
                        out.append((key, _mm(lhs(), w)))
                    pend.append(out)

            for j in (7, 5, 3, 1):
                tasks.append((1, functools.partial(task, j), {tl[4][0] for tl in bt}))

        def anchor(v):
            ps[nt + z2, 0:8, :] = v

        def sm_max():
            assert left["s", nt - 1] == 0
            res["mx"] = jnp.broadcast_to(jnp.max(res["m"], axis=-1, keepdims=True), (8, _L))

        def sm_exp(c):
            if c >= 4 and c % 2 == 0:
                anchor(res["l", c - 4])
            e = jnp.exp(ps[c, pl.ds(srow, 8), :] - res["mx"])
            es[c] = e
            res["l", c] = e if c == 0 else res["l", c - 1] + e
            if c == nt - 1:
                es[nt] = jnp.broadcast_to(1.0 / jnp.sum(res["l", c], axis=-1, keepdims=True), (8, _L))

        def fin(t):
            finish_o(t, 1 - g % 2, False)

        extra = {}
        if not last:
            extra[n_k + 4 * _SM_MAX] = sm_max
            for c in range(nt):
                extra[n_k + 4 * _SM_EXP + c] = functools.partial(sm_exp, c)
        for t in range(_KT):
            extra[4 + (1 if last else 8) * t] = functools.partial(fin, t)
        for i in sorted(extra, reverse=True):
            tasks.insert(i, (0, extra[i], ()))

        blocks = [(r, c) for r in range(0, hr, nj) for c in range(on_mxu(r // hl, last), nt)]
        total, span = sum(w for w, _, _ in tasks), len(blocks) - (_END_L if last else _END)
        hist, done, acc = [], 0, None
        for step, (r, c) in enumerate(blocks):
            ev = _EVERY_L if last else _EVERY
            if step % ev == 0:
                run = []
                while tasks and done * span < (step + ev) * total:
                    run.append(tasks.pop(0))
                    done += run[-1][0]
                if len(hist) > lag:
                    old = pltpu.bitcast(hist[-1 - lag], _U32)
                    kinds = set().union(*(k for _, _, k in run))
                    for a in range(2 * nj):
                        v = old[8 * a:8 * a + 8]
                        if kinds & {"s", "x"}:
                            ar[dm0 + z, a] = v
                        if "q" in kinds:
                            wq[d // 16 + z, a] = v
                        if "o" in kinds:
                            wo[_NG * hr + z, a] = v
                retire(_RETIRE)
                for _, fn, _ in run:
                    fn()
            pb = ps[c, pl.ds(prow + (16 * r) // _DH, 8, stride=0), :]
            pb = jnp.concatenate([pb] * (2 * nj), axis=0)
            vv = mat(varr, r, nj, [c]) if r < hr - hx else mat(xarr, r - (hr - hx), nj, [c])
            t = vv.astype(_F32) * pb
            acc = t if acc is None else acc + t
            hist.append(acc)
            if c == nt - 1:
                oacc[pl.ds(pl.multiple_of(_GR * (g % 2) + 16 * r, 8), 16 * nj), :] = acc
                acc = None
        assert not tasks
        retire(0)

    def layer(i, x):
        first = jnp.maximum(1 - i, 0)
        u, rs = _layernorm(x)
        u = _lhs(u)
        es[nt + 1] = rs
        u_ref[...] = pltpu.bitcast(u, _U32)
        xa_ref[...] = jnp.zeros_like(xa_ref)
        pl.loop(0, first)(lambda _: advance(-1))
        set_q(_mm(u, mat(wq, 0, d // 16, range(_KT))))
        q1 = _mm(u, mat(wq, 0, d // 16, range(_KT, 2 * _KT)))
        s = _mm(_bf(q_ref[...]), mat(ar, 0, hr, range(nt))) * (_DH ** -0.5)
        exp_sum(lambda c: s[:, c * _L:(c + 1) * _L], jnp.max(s, axis=-1, keepdims=True))
        set_q(q1)

        lax.fori_loop(0, _NG - 1, lambda g, _: group_body(first, g), None)
        group_body(first, _NG - 1 + z_ref[0], last=True)

        for t in range(_KT):
            finish_o(t, (_NG - 1) % 2, True)
        a = xa_ref[...] + _mm(_bf(ol_ref[...]), mat(wo, (_NG - 1) * hr, hr, range(d // _L)))
        x = _rb(x + _rb(a))
        pl.when(first > 0)(lambda: advance(_NG))
        u, rs = _layernorm(x)
        h = _mm(_lhs(u), mat(w1, 0, w1.shape[0], range(w1.shape[1])))
        h = h * jnp.concatenate([rs] * w1.shape[1], axis=1)
        h = _gelu(_rb(_rb(h) + b1_ref[...].astype(_F32)[None]))
        pl.when(first > 0)(lambda: advance(_NG + 1))
        h = _lhs(h)
        f = _mm(h[:, :16 * w2a], mat(w2, 0, w2a, range(d // _L)))
        pl.when(first > 0)(lambda: advance(_NG + 2))
        f = f + _mm(h[:, 16 * w2a:], mat(w2, w2a, 2 * hl, range(d // _L)))
        return _rb(x + _rb(_rb(f) + b2_ref[...].astype(_F32)[None]))

    x = lax.fori_loop(0, 2, layer, jnp.broadcast_to(x_ref[0].astype(_F32), (8, d)))
    o_ref[0] = x[0:1].astype(o_ref.dtype)


@jax.jit
def pallas_interleave_layers__sliding_block_cached__dense_activation_gelu__decode_kernel(
    A_x: jax.Array,
    A_k_cache: jax.Array,
    A_v_cache: jax.Array,
    A_wq: jax.Array,
    A_wo: jax.Array,
    B_x: jax.Array,
    B_w1: jax.Array,
    B_b1: jax.Array,
    B_w2: jax.Array,
    B_b2: jax.Array,
):
    d, f = B_w1.shape
    sk = A_k_cache.shape[2]
    w = min(4096, max(256, sk // 4))
    rows = _HQ * _DH
    kt = jnp.swapaxes(A_k_cache, 2, 3).reshape(rows, sk)
    vt = jnp.swapaxes(A_v_cache, 2, 3).reshape(rows, sk)

    def tiled(a):
        r, c = a.shape
        return a.reshape(r // 16, 2, 8, c // _L, _L).transpose(0, 1, 3, 2, 4)

    def buf(r, c, extra=0):
        return pltpu.VMEM((r // 16 + extra, c // _L, 16, _L), _BF)

    vm = pl.BlockSpec(memory_space=pltpu.VMEM)
    hbm = pl.BlockSpec(memory_space=pl.ANY)
    return pl.pallas_call(
        functools.partial(_kernel, start=(sk - w) // _L, nt=w // _L),
        out_shape=jax.ShapeDtypeStruct(A_x.shape, A_x.dtype),
        in_specs=[vm, vm, vm] + [hbm] * 6,
        out_specs=vm,
        scratch_shapes=[
            buf(rows + _NX * _NG * _L, w, 1),
            buf(rows - _NX * _NG * _L, w),
            buf(d, rows, 1),
            buf(rows, d, 1),
            buf(d, f),
            buf(f, d),
            pltpu.VMEM((w // _L + 1, 16, _L), _F32),
            pltpu.VMEM((w // _L + 2, 8, _L), _F32),
            pltpu.VMEM((8, d), _U32),
            pltpu.VMEM((8, _GR), _U32),
            pltpu.VMEM((8, _GR), _U32),
            pltpu.VMEM((2 * _GR, _L), _F32),
            pltpu.VMEM((_NX, 8, _L), _F32),
            pltpu.VMEM((8, d), _F32),
            pltpu.SMEM((2,), jnp.int32),
            pltpu.SemaphoreType.DMA((6 * _NG + 10,)),
        ],
        compiler_params=pltpu.CompilerParams(vmem_limit_bytes=126 * 2**20),
        name="attn_ffn_x2",
    )(A_x, B_b1, B_b2, *map(tiled, (kt, vt, A_wq, A_wo, B_w1, B_w2)))
```

```python
import functools

import jax
import jax.numpy as jnp
from jax import lax
import jax.experimental.pallas as pl
import jax.experimental.pallas.tpu as pltpu

_HQ, _DH = 32, 192
_L = 128
_GH = 4
_NG = _HQ // _GH
_GR = _GH * _DH
_KT = _GR // _L
_BF, _F32, _U32 = jnp.bfloat16, jnp.float32, jnp.uint32

_NX = 2
_XC, _XL = 32, 64
_NJ = 2
_EVERY, _EVERY_L = 6, 8
_END, _END_L = 16, 4
_LAG, _RETIRE = 8, 5
_SM_MAX, _SM_EXP = 6, 8


def _layernorm(x):
    m = jnp.mean(x, axis=-1, keepdims=True)
    d = x - m
    v = jnp.mean(d * d, axis=-1, keepdims=True)
    return d, jnp.broadcast_to(1.0 / jnp.sqrt(v + 1e-5), (x.shape[0], _L))


def _gelu(x):
    c = 0.7978845608028654
    return 0.5 * x * (1.0 + jnp.tanh(c * (x + 0.044715 * (x * x * x))))


def _rb(a):
    return a.astype(_BF).astype(_F32)


def _bf(a):
    return pltpu.bitcast(a, _BF)


def _lhs(a):
    return jnp.concatenate([a, a], axis=0).astype(_BF)


def _mm(a, b):
    return jnp.dot(a, b, preferred_element_type=_F32)[:8]


def _kernel(x_ref, b1_ref, b2_ref, k_hbm, v_hbm, wq_hbm, wo_hbm, w1_hbm, w2_hbm, o_ref,
            ar_b, vb_b, wq_b, wo_b, w1_b, w2_b, ps, es, u_ref, q_ref, ol_ref, oacc, ox_ref, xa_ref, z_ref, sem, *, start, nt):
    ar, vb, wq, wo, w1, w2 = (r.bitcast(_U32) for r in (ar_b, vb_b, wq_b, wo_b, w1_b, w2_b))
    nj, nx, lag = _NJ, _NX, _LAG
    d = x_ref.shape[-1]
    hr, hl = _GR // 16, _L // 16
    vx0 = _NG * hr
    hx = nx * hl
    dm0 = vx0 + _NG * hx

    w2a = w2_b.shape[0] - 2 * hl

    def copies(g):
        out = []

        def cp(src, r0, c0, dst, d0, n, i):
            nc = src.shape[2] - c0
            for h in range(2):
                out.append(pltpu.make_async_copy(
                    src.at[pl.ds(r0, n), h, pl.ds(c0, nc)],
                    dst.at[pl.ds(d0, n), pl.ds(0, nc), pl.ds(8 * h, 8)], sem.at[2 * i + h]))

        if g < 0:
            cp(wq_hbm, 0, 0, wq_b, 0, d // 16, 3)
        if g + 1 < _NG:
            cp(k_hbm, (g + 1) * hr, start, ar_b, (g + 1) * hr, hr, 3 * g + 7)
        if 0 <= g < _NG:
            cp(v_hbm, g * hr, start, vb_b, g * (hr - hx), hr - hx, 3 * g + 5)
            cp(v_hbm, (g + 1) * hr - hx, start, ar_b, vx0 + g * hx, hx, 3 * g + 6)
        if g == 0:
            cp(wo_hbm, 0, 0, wo_b, 0, _NG * hr, 0)
        if g == _NG:
            cp(w1_hbm, 0, 0, w1_b, 0, w1_b.shape[0], 1)
        if g == _NG + 1:
            cp(w2_hbm, 0, 0, w2_b, 0, w2a, 2)
        if g == _NG + 2:
            cp(w2_hbm, w2a, 0, w2_b, w2a, w2_b.shape[0] - w2a, 3 * _NG + 4)
        return out

    def mat(ref, r0, n, cols):
        return jnp.concatenate([_bf(ref[pl.ds(r0, n), c].reshape(8 * n, _L)) for c in cols], axis=1)

    def advance(g):
        for c in copies(g):
            c.wait()
        for c in copies(g + 2):
            c.start()

    for g in (-1, 0):
        for c in copies(g):
            c.start()

    oacc[...] = jnp.zeros_like(oacc)
    ox_ref[...] = jnp.zeros_like(ox_ref)
    z_ref[0] = 0
    z_ref[1] = 0

    def set_q(q):
        q = q * jnp.concatenate([es[nt + 1]] * _KT, axis=1)
        row = lax.broadcasted_iota(jnp.int32, q.shape, 0)
        col = lax.broadcasted_iota(jnp.int32, q.shape, 1)
        diag = (col >= row * _DH) & (col < (row + 1) * _DH)
        q_ref[...] = pltpu.bitcast(_lhs(jnp.where(diag, q, 0.0)), _U32)

    def exp_sum(s_of, m):
        l = None
        for c in range(nt):
            e = jnp.exp(s_of(c) - m)
            es[c] = e
            l = e if l is None else l + e
        r = jnp.broadcast_to(1.0 / jnp.sum(l, axis=-1, keepdims=True), (8, _L))
        es[nt] = r
        return r

    def on_mxu(t, last):
        return min(max((_XL if last else _XC) - (_KT - 1 - t) * nt, 0), nt)

    def finish_o(t, slot, last):
        a = None
        if on_mxu(t, last) < nt:
            a = oacc[pl.ds(pl.multiple_of(slot * _GR + t * _L, 8), _L), :].T
            a = jnp.sum(a.reshape(_L // 8, 8, _L), axis=0)
        if on_mxu(t, last):
            head = (t * _L + lax.broadcasted_iota(jnp.int32, (8, _L), 1)
                    - _DH * lax.broadcasted_iota(jnp.int32, (8, _L), 0))
            b = jnp.where((head >= 0) & (head < _DH), ox_ref[t - (_KT - nx)], 0.0)
            a = b if a is None else a + b
        o = jnp.sum(a, axis=0, keepdims=True)
        ol_ref[:, t * _L:(t + 1) * _L] = pltpu.bitcast(_lhs(jnp.broadcast_to(o, (8, _L))), _U32)

    def group_body(first, g, last=False):
        @pl.loop(0, first)
        def _(_):
            for j in ([_NG - 1] if last else range(_NG - 1)):
                pl.when(g == j)(functools.partial(advance, j))

            tu = 8

            @pl.loop(0, (_XL if last else _XC) // tu)
            def _(cb):
                at = [(vx0 + g * hx + (nx - 1 - (cb * tu) // nt) * hl, (cb * tu) % nt + c) for c in range(tu)]
                tr = [mat(ar, r, hl, [c]).T for r, c in at]
                for (r, c), a in zip(at, tr):
                    ar[pl.ds(r, hl), c] = pltpu.bitcast(a, _U32).reshape(hl, 8, _L)

        z, z2 = z_ref[0], z_ref[1]
        prow = pl.multiple_of(8 * z, 8)
        srow = pl.multiple_of(8 + 8 * z, 8)
        krow = (g + 1) * hr
        orow = jnp.maximum(g - 1, 0) * hr
        qcol = jnp.minimum(g + 2, _NG - 1) * _KT
        for c in range(nt):
            p = es[c] * es[nt]
            if c < on_mxu(_KT - 1, last):
                ps[c, pl.ds(prow, 8), :] = p
            for h in range(_GH):
                if c >= on_mxu(h * _DH // _L, last):
                    ps[c, pl.ds(pl.multiple_of(prow + 16 + 8 * h, 8), 8), :] = jnp.broadcast_to(p[h:h + 1], (8, _L))

        tiles = []
        karr, xarr = ar.at[pl.ds(krow, hr)], ar.at[pl.ds(vx0 + g * hx, hx)]
        varr = vb.at[pl.ds(g * (hr - hx), hr - hx)]
        for cb in range(0, 0 if last else nt, 4):
            for t in range(_KT):
                for c in range(cb, cb + 4):
                    tiles.append((karr, t, c, lambda t=t: _bf(q_ref[:, t * _L:(t + 1) * _L]), ("s", c)))
        n_k = len(tiles)
        for c in range(nt):
            for t in range(nx):
                if c < on_mxu(_KT - nx + t, last):
                    tiles.append((xarr, t, c, lambda c=c: _lhs(ps[c, pl.ds(prow, 8), :]), ("x", t)))
        for n in range(0 if last else _KT):
            for t in range(d // _L):
                tiles.append((wq.at[:, pl.ds(qcol, _KT)], t, n, lambda t=t: _bf(u_ref[:, t * _L:(t + 1) * _L]), ("q", n)))
        for n in range(d // _L):
            for t in range(_KT):
                tiles.append((wo.at[pl.ds(orow, hr)], t, n, lambda t=t: _bf(ol_ref[:, t * _L:(t + 1) * _L]),
                              ("o", n)))
        left = {}
        for tl in tiles:
            left[tl[4]] = left.get(tl[4], 0) + 1
        pend, res, qs = [], {}, {}

        def retire(n):
            while len(pend) > n:
                batch = pend.pop(0)
                for key, r in batch:
                    res[key] = r if key not in res else res[key] + r
                    left[key] -= 1
                    if left[key]:
                        continue
                    kind, i = key
                    cols = slice(i * _L, (i + 1) * _L)
                    if kind == "s":
                        sc = res[key] * (_DH ** -0.5)
                        ps[i, pl.ds(srow, 8), :] = sc
                        res["m"] = sc if i == 0 else jnp.maximum(res["m"], sc)
                    elif kind == "q":
                        qs[i] = res[key]
                        if len(qs) == _KT:
                            set_q(jnp.concatenate([qs[j] for j in range(_KT)], axis=1))
                    elif kind == "o":
                        xa_ref[:, cols] += jnp.where(g > 0, res[key], 0.0)
                    else:
                        ox_ref[i] = res[key]
                key = batch[-1][0]
                ps[nt + z2, 8:16, :] = res[key]

        tasks = []
        for b in range(0, len(tiles), 4):
            bt = tiles[b:b + 4]
            rows = [[None] * 8 for _ in bt]

            def task(j, bt=bt, rows=rows):
                for jj in (j, j - 1):
                    for r, (ref, t, c, *_) in zip(rows, bt):
                        r[jj] = ref[t * hl + jj, c]
                if j == 1:
                    out = []
                    for r, (_, _, _, lhs, key) in zip(rows, bt):
                        w = _bf(jnp.concatenate(r, axis=0))
                        out.append((key, _mm(lhs(), w)))
                    pend.append(out)

            for j in (7, 5, 3, 1):
                tasks.append((1, functools.partial(task, j), {tl[4][0] for tl in bt}))

        def anchor(v):
            ps[nt + z2, 0:8, :] = v

        def sm_max():
            assert left["s", nt - 1] == 0
            res["mx"] = jnp.broadcast_to(jnp.max(res["m"], axis=-1, keepdims=True), (8, _L))

        def sm_exp(c):
            if c >= 4 and c % 2 == 0:
                anchor(res["l", c - 4])
            e = jnp.exp(ps[c, pl.ds(srow, 8), :] - res["mx"])
            es[c] = e
            res["l", c] = e if c == 0 else res["l", c - 1] + e
            if c == nt - 1:
                es[nt] = jnp.broadcast_to(1.0 / jnp.sum(res["l", c], axis=-1, keepdims=True), (8, _L))

        def fin(t):
            finish_o(t, 1 - g % 2, False)

        extra = {}
        if not last:
            extra[n_k + 4 * _SM_MAX] = sm_max
            for c in range(nt):
                extra[n_k + 4 * _SM_EXP + c] = functools.partial(sm_exp, c)
        for t in range(_KT):
            extra[4 + (1 if last else 8) * t] = functools.partial(fin, t)
        for i in sorted(extra, reverse=True):
            tasks.insert(i, (0, extra[i], ()))

        blocks = [(r, c) for r in range(0, hr, nj) for c in range(on_mxu(r // hl, last), nt)]
        total, span = sum(w for w, _, _ in tasks), len(blocks) - (_END_L if last else _END)
        hist, done, acc = [], 0, None
        for step, (r, c) in enumerate(blocks):
            ev = _EVERY_L if last else _EVERY
            if step % ev == 0:
                run = []
                while tasks and done * span < (step + ev) * total:
                    run.append(tasks.pop(0))
                    done += run[-1][0]
                if len(hist) > lag:
                    old = pltpu.bitcast(hist[-1 - lag], _U32)
                    kinds = set().union(*(k for _, _, k in run))
                    for a in range(2 * nj):
                        v = old[8 * a:8 * a + 8]
                        if kinds & {"s", "x"}:
                            ar[dm0 + z, a] = v
                        if "q" in kinds:
                            wq[d // 16 + z, a] = v
                        if "o" in kinds:
                            wo[_NG * hr + z, a] = v
                retire(_RETIRE)
                for _, fn, _ in run:
                    fn()
            pb = ps[c, pl.ds(pl.multiple_of(prow + 16 + 8 * ((16 * r) // _DH), 8), 8), :]
            pb = jnp.concatenate([pb] * (2 * nj), axis=0)
            vv = mat(varr, r, nj, [c]) if r < hr - hx else mat(xarr, r - (hr - hx), nj, [c])
            t = vv.astype(_F32) * pb
            acc = t if acc is None else acc + t
            hist.append(acc)
            if c == nt - 1:
                oacc[pl.ds(pl.multiple_of(_GR * (g % 2) + 16 * r, 8), 16 * nj), :] = acc
                acc = None
        assert not tasks
        retire(0)

    def layer(i, x):
        first = jnp.maximum(1 - i, 0)
        u, rs = _layernorm(x)
        u = _lhs(u)
        es[nt + 1] = rs
        u_ref[...] = pltpu.bitcast(u, _U32)
        xa_ref[...] = jnp.zeros_like(xa_ref)
        pl.loop(0, first)(lambda _: advance(-1))
        set_q(_mm(u, mat(wq, 0, d // 16, range(_KT))))
        q1 = _mm(u, mat(wq, 0, d // 16, range(_KT, 2 * _KT)))
        s = _mm(_bf(q_ref[...]), mat(ar, 0, hr, range(nt))) * (_DH ** -0.5)
        exp_sum(lambda c: s[:, c * _L:(c + 1) * _L], jnp.max(s, axis=-1, keepdims=True))
        set_q(q1)

        lax.fori_loop(0, _NG - 1, lambda g, _: group_body(first, g), None)
        group_body(first, _NG - 1 + z_ref[0], last=True)

        for t in range(_KT):
            finish_o(t, (_NG - 1) % 2, True)
        a = xa_ref[...] + _mm(_bf(ol_ref[...]), mat(wo, (_NG - 1) * hr, hr, range(d // _L)))
        x = _rb(x + _rb(a))
        pl.when(first > 0)(lambda: advance(_NG))
        u, rs = _layernorm(x)
        h = _mm(_lhs(u), mat(w1, 0, w1.shape[0], range(w1.shape[1])))
        h = h * jnp.concatenate([rs] * w1.shape[1], axis=1)
        h = _gelu(_rb(_rb(h) + b1_ref[...].astype(_F32)[None]))
        pl.when(first > 0)(lambda: advance(_NG + 1))
        h = _lhs(h)
        f = _mm(h[:, :16 * w2a], mat(w2, 0, w2a, range(d // _L)))
        pl.when(first > 0)(lambda: advance(_NG + 2))
        f = f + _mm(h[:, 16 * w2a:], mat(w2, w2a, 2 * hl, range(d // _L)))
        return _rb(x + _rb(_rb(f) + b2_ref[...].astype(_F32)[None]))

    x = lax.fori_loop(0, 2, layer, jnp.broadcast_to(x_ref[0].astype(_F32), (8, d)))
    o_ref[0] = x[0:1].astype(o_ref.dtype)


@jax.jit
def pallas_interleave_layers__sliding_block_cached__dense_activation_gelu__decode_kernel(
    A_x: jax.Array,
    A_k_cache: jax.Array,
    A_v_cache: jax.Array,
    A_wq: jax.Array,
    A_wo: jax.Array,
    B_x: jax.Array,
    B_w1: jax.Array,
    B_b1: jax.Array,
    B_w2: jax.Array,
    B_b2: jax.Array,
):
    d, f = B_w1.shape
    sk = A_k_cache.shape[2]
    w = min(4096, max(256, sk // 4))
    rows = _HQ * _DH
    kt = jnp.swapaxes(A_k_cache, 2, 3).reshape(rows, sk)
    vt = jnp.swapaxes(A_v_cache, 2, 3).reshape(rows, sk)

    def tiled(a):
        r, c = a.shape
        return a.reshape(r // 16, 2, 8, c // _L, _L).transpose(0, 1, 3, 2, 4)

    def buf(r, c, extra=0):
        return pltpu.VMEM((r // 16 + extra, c // _L, 16, _L), _BF)

    vm = pl.BlockSpec(memory_space=pltpu.VMEM)
    hbm = pl.BlockSpec(memory_space=pl.ANY)
    return pl.pallas_call(
        functools.partial(_kernel, start=(sk - w) // _L, nt=w // _L),
        out_shape=jax.ShapeDtypeStruct(A_x.shape, A_x.dtype),
        in_specs=[vm, vm, vm] + [hbm] * 6,
        out_specs=vm,
        scratch_shapes=[
            buf(rows + _NX * _NG * _L, w, 1),
            buf(rows - _NX * _NG * _L, w),
            buf(d, rows, 1),
            buf(rows, d, 1),
            buf(d, f),
            buf(f, d),
            pltpu.VMEM((w // _L + 1, 16 + 8 * _GH, _L), _F32),
            pltpu.VMEM((w // _L + 2, 8, _L), _F32),
            pltpu.VMEM((8, d), _U32),
            pltpu.VMEM((8, _GR), _U32),
            pltpu.VMEM((8, _GR), _U32),
            pltpu.VMEM((2 * _GR, _L), _F32),
            pltpu.VMEM((_NX, 8, _L), _F32),
            pltpu.VMEM((8, d), _F32),
            pltpu.SMEM((2,), jnp.int32),
            pltpu.SemaphoreType.DMA((6 * _NG + 10,)),
        ],
        compiler_params=pltpu.CompilerParams(vmem_limit_bytes=126 * 2**20),
        name="attn_ffn_x2",
    )(A_x, B_b1, B_b2, *map(tiled, (kt, vt, A_wq, A_wo, B_w1, B_w2)))
```
